```python
import jax
import jax.numpy as jnp

def _softmax(x, axis=-1):
    return jax.nn.softmax(x, axis=axis)

def _gelu(x):
    return jax.nn.gelu(x, approximate=True)

def _silu(x):
    return jax.nn.silu(x)

def _sigmoid(x):
    return jax.nn.sigmoid(x)

def _layernorm(x, axis=-1, eps=1e-05):
    m = jnp.mean(x, axis=axis, keepdims=True)
    v = jnp.var(x, axis=axis, keepdims=True)
    return (x - m) / jnp.sqrt(v + eps)

def _scatter_add(tgt, idx, src, axis=0):
    return tgt.at[idx].add(src)

def _segment_sum(src, seg, n):
    return jax.ops.segment_sum(src, seg, n)

class _Rng:

    def __init__(self, key):
        self._k = key

    def _next(self):
        self._k, sub = jax.random.split(self._k)
        return sub

    def normal(self, shape):
        return jax.random.normal(self._next(), shape, dtype=jnp.bfloat16)

    def randint(self, lo, hi, shape):
        return jax.random.randint(self._next(), shape, lo, hi, dtype=jnp.int32)

    def uniform(self, shape, lo=0.0, hi=1.0):
        return jax.random.uniform(self._next(), shape, jnp.bfloat16, lo, hi)

    def permutation(self, n):
        return jax.random.permutation(self._next(), n)
kernel_name = 'adaLN_cond__spectral_gfnet__geglu_ffn__prompt'

def _fwd_setup_inputs():
    _rng = _Rng(jax.random.key(int.from_bytes(__import__("os").urandom(4), "little")))
    _w = lambda a: (lambda t: t.astype(jnp.bfloat16) if jnp.issubdtype(t.dtype, jnp.floating) else t)(jnp.asarray(a))

    def _A_setup():
        B, S, D = (1, 2048, 512)
        Df = D // 2 + 1
        return {'x': _w((lambda *s: _rng.normal(s) * 0.05)(B, S, D)), 'w_r': _w((lambda *s: _rng.normal(s) * 0.05)(S, Df) * 0.02), 'w_i': _w((lambda *s: _rng.normal(s) * 0.05)(S, Df) * 0.02)}
    _A_in = _A_setup()

    def _B_setup():
        B, S, D, F = (1, 2048, 512, 1792)
        return {'x': _w((lambda *s: _rng.normal(s) * 0.05)(B, S, D)), 'w_gate': _w((lambda *s: _rng.normal(s) * 0.05)(D, F)), 'w_up': _w((lambda *s: _rng.normal(s) * 0.05)(D, F)), 'w_down': _w((lambda *s: _rng.normal(s) * 0.05)(F, D))}
    _B_in = _B_setup()
    return {'A_x': _A_in['x'], 'A_w_r': _A_in['w_r'], 'A_w_i': _A_in['w_i'], 'B_x': _B_in['x'], 'B_w_gate': _B_in['w_gate'], 'B_w_up': _B_in['w_up'], 'B_w_down': _B_in['w_down'], 'c': _w((lambda *s: _rng.normal(s) * 0.05)(1, 512)), 'w_mod': _w((lambda *s: _rng.normal(s) * 0.05)(512, 6 * 512) * 512 ** (-0.5))}

def _fwd_reference(A_x, A_w_r, A_w_i, B_x, B_w_gate, B_w_up, B_w_down, c, w_mod):

    def _A_ref(x, w_r, w_i):
        B, S, D = x.shape
        X = (lambda x, axes=(-2, -1): jnp.fft.rfft2(x.astype(jnp.float32), axes=axes))(x, axes=(-2, -1))
        W = w_r + 1j * w_i
        X = X * W
        y = (lambda x, s, axes=(-2, -1): jnp.fft.irfft2(x, s=s, axes=axes).astype(jnp.bfloat16))(X, (S, D), axes=(-2, -1))
        return y

    def _B_ref(x, w_gate, w_up, w_down):
        return _gelu(x @ w_gate) * (x @ w_up) @ w_down
    x = A_x
    mod = (_silu(c) @ w_mod).reshape(c.shape[0], 6, 1, -1)
    sa, ca, ga, sb, cb, gb = (mod[:, 0].copy(), mod[:, 1].copy(), mod[:, 2].copy(), mod[:, 3].copy(), mod[:, 4].copy(), mod[:, 5].copy())
    h = _layernorm(x, axis=-1) * (1 + ca) + sa
    x = x + ga * _A_ref(h, A_w_r, A_w_i)
    h = _layernorm(x, axis=-1) * (1 + cb) + sb
    x = x + gb * _B_ref(h, B_w_gate, B_w_up, B_w_down)
    return x

def setup_inputs():
    _inp = _fwd_setup_inputs()
    _gk = jax.random.fold_in(jax.random.key(int.from_bytes(__import__("os").urandom(4), "little")), 2 ** 31 - 1)
    _shapes = [[1, 2048, 512]]
    _dtypes = ['bfloat16']
    _gks = jax.random.split(_gk, len(_shapes))
    _gs = [jax.random.normal(k, s, dtype=jnp.dtype(d)) * 0.05 for k, s, d in zip(_gks, _shapes, _dtypes)]
    _inp['grad_out'] = _gs[0]
    return _inp

def reference(A_x, A_w_r, A_w_i, B_w_gate, B_w_up, B_w_down, c, w_mod, B_x, grad_out):
    _const = dict(B_x=B_x)

    def _f(*_d):
        return _fwd_reference(**{'A_x': _d[0], 'A_w_r': _d[1], 'A_w_i': _d[2], 'B_w_gate': _d[3], 'B_w_up': _d[4], 'B_w_down': _d[5], 'c': _d[6], 'w_mod': _d[7], **_const})
    _out, _vjp = jax.vjp(_f, A_x, A_w_r, A_w_i, B_w_gate, B_w_up, B_w_down, c, w_mod)
    _grads = _vjp(grad_out)
    _out0 = jnp.asarray(_out)
    return (_out0, *[jnp.asarray(_g) for _g in _grads])
```

```python
import functools
import math

import numpy as np
import jax
import jax.numpy as jnp
import jax.experimental.pallas as pl
import jax.experimental.pallas.tpu as pltpu

S, D, F = 2048, 512, 1792
N1, N2 = 32, 64
H = 256
NTILE = S // (2 * H)
Q = 128
R = 16
JH = F // 256
BF, F32, U32 = jnp.bfloat16, jnp.float32, jnp.uint32
EPS = 1e-5
G0 = math.sqrt(2.0 / math.pi)
G1 = 0.044715 * G0


def _constants():
    r = np.arange(128)[:, None].astype(np.float64)
    l = np.arange(128)[None, :]
    ev = l % 2 == 0
    th = lambda k: 2.0 * np.pi * k * r / D
    k_im = 2.0 * ((l - 1) % 128)
    d0 = np.where(ev, np.cos(th(2.0 * l)), -np.sin(th(k_im)))
    d2 = np.where(ev, -np.sin(th(k_im)), np.cos(th(2.0 * l)))
    odd = th(2.0 * l + 1.0)
    p_re, p_im = np.cos(odd), -np.sin(odd)
    q_re = np.where(ev, -np.sin(odd), np.sin(odd))
    q_im = np.where(ev, -np.cos(odd), np.cos(odd))
    dmat = np.stack([d0, d2, p_re, q_re, p_im, q_im])
    b = np.arange(N2)[None, None, :]
    bp = np.arange(N2)[None, :, None]
    ap = np.arange(N1)[:, None, None]
    phi = 2.0 * np.pi * ((b * (ap + N1 * bp)) % S) / S
    c, s = np.cos(phi), np.sin(phi)
    col_re = np.concatenate([c, -s], axis=1).reshape(N1, 2 * N2, N2 // 8, 1, 8)
    col_im = np.concatenate([s, c], axis=1).reshape(N1, 2 * N2, N2 // 8, 1, 8)
    mf = np.concatenate([col_re, col_im], axis=3).reshape(N1, 2 * N2, 2 * N2)
    a = np.arange(128)[:, None]
    ok = (a < N1) & (l < N1)
    fc = np.where(ok, np.cos(2.0 * np.pi * ((a * l) % N1) / N1), 0.0)
    fs = np.where(ok, -np.sin(2.0 * np.pi * ((a * l) % N1) / N1), 0.0)
    tw = 2.0 * np.pi * np.arange(N2)[:, None] * l / S
    twid = np.stack([np.cos(tw), np.sin(tw)]).astype(np.float32)
    dmat = np.concatenate([dmat, fc[None], fs[None]]).astype(np.float32).astype(jnp.bfloat16)
    return dmat, mf.astype(np.float32).astype(jnp.bfloat16), twid


_DMAT, _MF, _TWID = _constants()
_SPARE = np.array([0, S, N1, 2 * JH, 6, D, 0, S // 128], np.int32)


def _dot(a, b):
    return jax.lax.dot_general(a, b, (((1,), (0,)), ((), ())), preferred_element_type=F32)


def _dot_nt(a, b):
    return jax.lax.dot_general(a, b, (((1,), (1,)), ((), ())), preferred_element_type=F32)


def _cat(xs, axis=1):
    return jnp.concatenate(xs, axis=axis)


def _tiles(v):
    return [v[:, 128 * t:128 * t + 128] for t in range(v.shape[1] // 128)]


def _alpha(a11, a12, a21, a22):
    return [a11 + a22, a21 + a22, a11, a22, a11 + a12, a21 - a11, a12 - a22]


def _beta(b11, b12, b21, b22):
    return [b11 + b22, b11, b12 - b22, b21 - b11, b22, b11 + b12, b21 + b22]


def _gamma(c11, c12, c21, c22):
    return [c11 + c22, c21 - c22, c12 + c22, c11 + c21, c12 - c11, c22, c11]


def _alpha_t(p):
    return [p[0] + p[2] + p[4] - p[5], p[4] + p[6], p[1] + p[5], p[0] + p[1] + p[3] - p[6]]


def _beta_t(q):
    return [q[0] + q[1] - q[3] + q[5], q[2] + q[5], q[3] + q[6], q[0] - q[2] + q[4] + q[6]]


def _gamma_t(m):
    return [m[0] + m[3] - m[4] + m[6], m[2] + m[4], m[1] + m[3], m[0] - m[1] + m[2] + m[5]]


_PLAIN = {_alpha: {2: 0, 3: 3}, _beta: {1: 0, 4: 3}, _gamma: {5: 3, 6: 0}}


def aligned(v, n):
    return v if isinstance(v, int) else pl.multiple_of(v, n)


def _bf(words):
    return pltpu.bitcast(words, BF)


def _twiddle(z, k, n, sign):
    re, im = z
    k %= n
    if k == 0:
        return z
    if 8 * k == n or 8 * k == 3 * n:
        h = math.sqrt(0.5)
        if 8 * k == n:
            return ((re - im) * h, (re + im) * h) if sign > 0 else ((re + im) * h, (im - re) * h)
        return ((re + im) * (-h), (re - im) * h) if sign > 0 else ((im - re) * h, (re + im) * (-h))
    c, s = math.cos(2.0 * math.pi * k / n), sign * math.sin(2.0 * math.pi * k / n)
    return (re * c - im * s, re * s + im * c)


def _dft(z, sign):
    n = len(z)
    if n == 1:
        return z
    if n == 2:
        return [(z[0][0] + z[1][0], z[0][1] + z[1][1]), (z[0][0] - z[1][0], z[0][1] - z[1][1])]
    u, v, w = _dft(z[0::2], sign), _dft(z[1::4], sign), _dft(z[3::4], sign)
    out = [None] * n
    q = n // 4
    for k in range(q):
        a, b = _twiddle(v[k], k, n, sign), _twiddle(w[k], 3 * k, n, sign)
        sr, si = a[0] + b[0], a[1] + b[1]
        dr, di = a[0] - b[0], a[1] - b[1]
        out[k] = (u[k][0] + sr, u[k][1] + si)
        out[k + 2 * q] = (u[k][0] - sr, u[k][1] - si)
        plus = (u[k + q][0] - di, u[k + q][1] + dr)
        minus = (u[k + q][0] + di, u[k + q][1] - dr)
        out[k + q], out[k + 3 * q] = (plus, minus) if sign > 0 else (minus, plus)
    return out


def _rowsum(tiles):
    acc = tiles[0]
    for t in tiles[1:]:
        acc = acc + t
    return jnp.sum(acc, axis=1, keepdims=True)


def _colsum8(v):
    parts = [v[r:r + 8] for r in range(0, v.shape[0], 8)]
    while len(parts) > 1:
        parts = [parts[i] + parts[i + 1] for i in range(0, len(parts), 2)]
    return parts[0]


def _geglu(g, u, da):
    g2 = g * g
    cdf = 0.5 * jnp.tanh(g * (G0 + G1 * g2)) + 0.5
    ge = g * cdf
    dge = cdf + (ge * (1.0 - cdf)) * (2.0 * G0 + (6.0 * G1) * g2)
    return da * (u * dge), da * ge, ge * u


def _kernel(spare_ref, c_ref, twid_ref, x_hbm, do_hbm, wr_hbm, wi_hbm, wg_hbm, wu_hbm, wd_hbm, wm_hbm, dmat_hbm, mf_hbm,
            out_hbm, dx_hbm, dwr_hbm, dwi_hbm, dwg_hbm, dwu_hbm, dwd_hbm, dc_ref, dwm_hbm,
            x_v, do_v, wri_v, wgu_v, wd_v, wm_v, dmat_v, mf_v,
            dall, mi_v, scol, mod_v, bgu, bd, obuf, zbuf, vbuf, xs, wq, dwq, wn, xn, nyq,
            y1_v, st1, st2, ah, lt, act, da_v, out_v, dx_v, dx1_v, dwm_v, sums, dcacc, isem, osem):
    lane = jax.lax.broadcasted_iota(jnp.int32, (N2, 128), 1)
    lane_h = jax.lax.broadcasted_iota(jnp.int32, (H, 128), 1)
    even_h = (lane_h & 1) == 0
    sgn_h = (1 - 2 * (lane_h & 1)).astype(F32)

    dall32, bgu32, bd32, zbuf32, ah32, lt32, act32 = (
        r.bitcast(U32) for r in (dall, bgu, bd, zbuf, ah, lt, act))

    def wm_copy(b):
        return pltpu.make_async_copy(wm_hbm.at[:, pl.ds(D * b, D)], wm_v.at[b], isem.at[b])

    def row_copy(src, dst, base, i):
        rows = pl.ds(2 * H * i, 2 * H)
        return pltpu.make_async_copy(src.at[rows], dst.at[rows], isem.at[base + i])

    x_copy = lambda i: row_copy(x_hbm, x_v, 6, i)
    do_copy = lambda i: row_copy(do_hbm, do_v, 10, i)
    col_groups = [(j, min(j + 2, JH)) for j in range(0, JH, 2)]

    wd_copy = pltpu.make_async_copy(wd_hbm, wd_v, isem.at[23])
    wgu_copies = [pltpu.make_async_copy(src, wgu_v.at[w, pl.ds(0, D)], isem.at[14 + w])
                  for w, src in enumerate((wg_hbm, wu_hbm))]
    dmat_copy = pltpu.make_async_copy(dmat_hbm, dmat_v, isem.at[16])
    mf_copy = pltpu.make_async_copy(mf_hbm, mf_v, isem.at[17])
    wri_copies = [pltpu.make_async_copy(src, wri_v.at[k], isem.at[18 + k]) for k, src in enumerate((wr_hbm, wi_hbm))]

    for cp in [wm_copy(0), wm_copy(1), dmat_copy, x_copy(0)]:
        cp.start()

    cv = c_ref[...].astype(F32)
    sig = 1.0 / (1.0 + jnp.exp(-cv))
    s_row = (cv * sig).astype(BF).astype(F32)
    scol[0:D, :] = jnp.broadcast_to(s_row, (128, D)).T

    def mod_block(b):
        sc = scol[0:D, :]
        parts = [_colsum8(t.astype(F32) * sc) for t in _tiles(wm_v[b])]
        tot = jnp.sum(_cat(parts), axis=0, keepdims=True)
        mod_v[b] = jnp.broadcast_to(tot.astype(BF).astype(F32), (8, D))

    def mod_row(b):
        return mod_v[b, 0:1, :]

    sums[...] = jnp.zeros(sums.shape, F32)
    nyq[...] = jnp.zeros(nyq.shape, F32)
    wm_copy(0).wait()
    x_copy(1).start()
    mod_block(0)
    wm_copy(1).wait()
    mod_block(1)

    dmat_copy.wait()
    lane_d = jax.lax.broadcasted_iota(jnp.int32, (128, 128), 1)
    for k in range(6):
        m = dmat_v[k]
        scale = jnp.where(lane_d == 0, 1.0 / (S * D), 2.0 / (S * D)) if k == 0 else 2.0 / (S * D)
        ms = m.astype(F32) * scale
        dall[0, k] = m
        dall[1, k] = ms.astype(BF)
        dall[2, k] = m.astype(F32).T.astype(BF)
        dall[3, k] = ms.T.astype(BF)

    def after(ref, lead, val):
        rows = 8 * 4 // ref.dtype.itemsize
        idx = tuple(spare_ref[k] for k in lead[:-1]) + (pl.ds(pl.multiple_of(spare_ref[lead[-1]], rows), rows),)
        ref[idx + (slice(0, 128),)] = val[0:rows, 0:128].astype(ref.dtype)

    def d_forward(h, r0, a0, sel):
        n = h.shape[0]
        h0, h1, h2, h3 = _tiles(h)
        t0, t1 = h0 + h2, h1 + h3
        z0, z2 = t0 + t1, t0 - t1
        o0 = _dot(z0.astype(BF), dall[sel, 0])
        o2 = _dot(z2.astype(BF), dall[sel, 1])
        dd = _bf(_cat([_cat([dall32[sel, 2], dall32[sel, 3]], 0), _cat([dall32[sel, 4], dall32[sel, 5]], 0)]))
        odd = _dot(_cat([h0 - h2, h1 - h3]).astype(BF), dd)
        rows = pl.ds(r0, n)
        obuf[0, rows, :] = jnp.where(even_h[:n], o0, o2)
        obuf[1, rows, :] = odd[:, :128]
        obuf[2, rows, :] = pltpu.roll(jnp.where(even_h[:n], o2, o0), 127, 1)
        obuf[3, rows, :] = odd[:, 128:]
        ncol = jnp.sum(z0 * sgn_h[:n], axis=1, keepdims=True)
        acc = nyq[...]
        for t in range(n // N2):
            acc = jnp.where(lane == a0 + t, ncol[N2 * t:N2 * t + N2], acc)
        nyq[...] = acc

    def d_inverse(r0, n, a0, sel):
        rows = pl.ds(r0, n)
        re_e, im_e = obuf[0, rows, :], pltpu.roll(obuf[2, rows, :], 1, 1)
        z0 = _dot(jnp.where(even_h[:n], re_e, im_e).astype(BF), dall[sel, 0])
        z2 = _dot(jnp.where(even_h[:n], im_e, re_e).astype(BF), dall[sel, 1])
        dd = _bf(_cat([_cat([dall32[sel, 2], dall32[sel, 4]], 0), _cat([dall32[sel, 3], dall32[sel, 5]], 0)]))
        pq = _dot(_cat([obuf[1, rows, :], obuf[3, rows, :]]).astype(BF), dd)
        nq = nyq[...]
        ncol = _cat([jnp.sum(jnp.where(lane == a0 + t, nq, 0.0), axis=1, keepdims=True) for t in range(n // N2)], 0)
        z0 = z0 + ncol * sgn_h[:n]
        t0, t1 = z0 + z2, z0 - z2
        p, q = pq[:, :128], pq[:, 128:]
        return _cat([t0 + p, t1 + q, t0 - p, t1 - q])

    def radix_steps(load, store, sign):
        z = [None] * N1

        def step(first):
            for a in range(first, N1, 4):
                z[a] = load(a)
            if first == 3:
                for a, (re, im) in enumerate(_dft(z, sign)):
                    store(a, re, im)

        return [functools.partial(step, first) for first in (0, 2, 1, 3)] + [None]

    def radix_forward(t, g):
        rows = lambda a: slice(N2 * a + 8 * g, N2 * a + 8 * g + 8)

        def store(a, re, im):
            zbuf[t, a, 16 * g:16 * g + 16, :] = _cat([re, im], 0).astype(BF)

        return radix_steps(lambda a: (obuf[t, rows(a), :], obuf[2 + t, rows(a), :]), store, -1)

    def radix_inverse(t, g):
        def store(a, re, im):
            obuf[t, N2 * a + 8 * g:N2 * a + 8 * g + 8, :] = re
            obuf[2 + t, N2 * a + 8 * g:N2 * a + 8 * g + 8, :] = im

        return radix_steps(lambda a: (vbuf[t, a, 16 * g:16 * g + 8, :], vbuf[t, a, 16 * g + 8:16 * g + 16, :]), store, 1)

    after_obuf = lambda v: after(obuf, (0, 1), v)
    after_vbuf = lambda v: after(vbuf, (0, 2, 0), v)

    def interleave8(re, im):
        return _cat([v[8 * g:8 * g + 8] for g in range(N2 // 8) for v in (re, im)], 0)

    def nyq_forward():
        n = nyq[...].astype(BF)
        zr, zi = _dot(n, dmat_v[6]), _dot(n, dmat_v[7])
        tc, ts = twid_ref[0], twid_ref[1]
        xq = _dot(mf_v[0], interleave8(zr * tc + zi * ts, zi * tc - zr * ts).astype(BF))
        return xq[:N2], xq[N2:]

    def nyq_inverse(yr, yi):
        v = _dot(mi_v[0], _cat([yr, yi], 0).astype(BF))
        vr = _cat([v[16 * g:16 * g + 8] for g in range(N2 // 8)], 0)
        vi = _cat([v[16 * g + 8:16 * g + 16] for g in range(N2 // 8)], 0)
        tc, ts = twid_ref[0], twid_ref[1]
        nyq[...] = (_dot((vr * tc - vi * ts).astype(BF), dmat_v[6]) + _dot((vr * ts + vi * tc).astype(BF), dmat_v[7]))

    def unpack_pair(w):
        return pltpu.bitcast(w << 16, F32), pltpu.bitcast(w & jnp.uint32(0xFFFF0000), F32)

    UN = 16

    def s_forward(a):
        return _dot(mf_v[a], _bf(_cat([zbuf32[0, a], zbuf32[1, a]])))

    def s_inverse(a, yr, yi):
        v = _dot(mi_v[a], _cat([yr, yi], 0).astype(BF))
        vbuf[0, a] = v[:, :128]
        vbuf[1, a] = v[:, 128:]

    def da_chunk(i, between, group_start=lambda n: None):
        top, bot = pl.ds(aligned(2 * H * i, H), H), pl.ds(aligned(2 * H * i + H, H), H)
        gb = mod_row(5)
        dt, db = do_v[top, :].astype(F32) * gb, do_v[bot, :].astype(F32) * gb
        quads = [dt[:, :256], dt[:, 256:], db[:, :256], db[:, 256:]]
        lhs = [g.astype(BF) for g in _gamma(*quads)]
        for n, (j0, j1) in enumerate(col_groups):
            words = slice(64 * j0, 64 * j1)
            group_start(n)
            p = []
            for k in range(7):
                p.append(_dot_nt(lhs[k], _bf(_cat([bd32[k, 0, words, :], bd32[k, 1, words, :]]))))
                between(7 * n + k, p[k])
            for q, v in enumerate(_alpha_t(p)):
                for j, tile in enumerate(_tiles(v)):
                    da_v[JH * (q % 2) + j0 + j, top if q < 2 else bot, :] = tile.astype(BF)

    def operands(fn, w, blocks, axis):
        sums_f32 = fn(*[_cat([act[w, j, pl.ds(r, H), :].astype(F32) for j, r in blk], axis) for blk in blocks])
        out = []
        for k in range(7):
            if k in _PLAIN[fn]:
                half = lambda r: aligned(r // 2, H // 2)
                out.append(_bf(_cat([act32[w, j, pl.ds(half(r), H // 2), :] for j, r in blocks[_PLAIN[fn][k]]], axis)))
            else:
                out.append(sums_f32[k].astype(BF))
        return out

    def dw_blocks(w, j, between):
        blocks = [[(JH * (q % 2) + j, 2 * H * i + H * (q // 2)) for i in range(NTILE)] for q in range(4)]
        q = []
        for k, g in enumerate(operands(_gamma, w, blocks, 0)):
            q.append(_dot(_bf(_cat([lt32[w // 2, k, t] for t in range(2 * NTILE)])), g))
            between(k, q[k])
        return _beta_t(q)

    dwgu_copies = [pltpu.make_async_copy(wgu_v.at[w, pl.ds(0, D)], dst, osem.at[8 + w])
                   for w, dst in enumerate((dwg_hbm, dwu_hbm))]

    def dwgu_chunk(n, between):
        w, j = n // JH, n % JH
        for q, blk in enumerate(dw_blocks(w, j, between)):
            cols = pl.ds(pl.multiple_of(128 * (JH * (q % 2) + j), 128), 128)
            wgu_v[w, 256 * (q // 2):256 * (q // 2) + 256, cols] = blk.astype(BF)

    def dwd_copy(j, half):
        rows = pl.ds(pl.multiple_of((F // 2) * half + 128 * j, 128), 128)
        return pltpu.make_async_copy(wd_v.at[rows], dwd_hbm.at[rows], osem.at[13])

    def dwd_chunk(j, between):
        for q, blk in enumerate(dw_blocks(2, j, between)):
            rows = pl.ds(pl.multiple_of((F // 2) * (q % 2) + 128 * j, 128), 128)
            wd_v[rows, 256 * (q // 2):256 * (q // 2) + 256] = blk.T.astype(BF)

    def dwd_start(j):
        for half in range(2):
            dwd_copy(j, half).start()

    def shifted(between, n):
        return lambda k, val: between(7 * n + k, val)

    def half_rows(i, h):
        r0 = aligned(2 * H * i + H * h, H)
        return r0, pl.ds(r0, H), (2 * H * i + H * h) // N2

    def spread(work, tie, slots):
        def between(k, val):
            todo = work[k * len(work) // slots:(k + 1) * len(work) // slots]
            for n, thunk in enumerate(todo):
                if thunk is not None:
                    r = (n * val.shape[0] // len(todo)) // 16 * 16
                    tie(val[r:r + 16])
                    thunk()
        return between

    def ln1_step(i, carry):
        x_copy(i).wait()
        for n, later in enumerate(([x_copy(2), x_copy(3)], [wm_copy(5), do_copy(0), wd_copy], [], [mf_copy] + wri_copies)):
            if not later:
                continue

            @pl.when(i == n)
            def _():
                for cp in later:
                    cp.start()

        for part in range(2 * H // Q):
            r0 = pl.multiple_of(2 * H * i + Q * part, Q)
            rows = pl.ds(r0, Q)
            xv = x_v[rows, :].astype(F32)
            mu = _rowsum(_tiles(xv)) * (1.0 / D)
            xc = xv - mu
            rstd = jax.lax.rsqrt(_rowsum(_tiles(xc * xc)) * (1.0 / D) + EPS)
            st1[0, rows, :] = jnp.broadcast_to(mu, (Q, 128))
            st1[1, rows, :] = jnp.broadcast_to(rstd, (Q, 128))
            after(x_v, (1,), xc)
            d_forward((xc * rstd) * (1.0 + mod_row(1)) + mod_row(0), r0, (2 * H * i + Q * part) // N2, 0)
        return carry

    jax.lax.fori_loop(0, NTILE, ln1_step, 0)
    for cp in (wd_copy, wm_copy(5), do_copy(0)):
        cp.wait()
    for cp in [do_copy(1)] + wgu_copies:
        cp.start()
    mod_block(5)

    def beta_d(n):
        j0, j1 = col_groups[n]
        for t in range(2):
            quads = [wd_v[pl.ds((F // 2) * half + 128 * j0, 128 * (j1 - j0)), 128 * (c + t):128 * (c + t + 1)].astype(F32)
                     for half in range(2) for c in (0, 2)]
            for k, v in enumerate(_beta(*quads)):
                bd[k, t, 128 * j0:128 * j1, :] = v.astype(BF)

    groups = [(t, g) for t in range(2) for g in range(N2 // 8)]
    sub = jax.lax.broadcasted_iota(jnp.int32, (N2, 128), 0)

    def filter_prep(n):
        beta_d(n)
        if n != 3:
            return
        for cp in [mf_copy] + wri_copies:
            cp.wait()
        for a in range(N1):
            mi_v[a] = mf_v[a].T
        for k in range(2):
            for t in range(S // 128):
                words = pltpu.bitcast(wri_v[k, 0:256, 128 * t:128 * t + 128], U32)
                wq[k, t] = jnp.take_along_axis(words, (lane_d >> 2) + N1 * (lane_d & 3), axis=1).T
            last = wri_v[k, 256:257, :].astype(F32)
            rep = _cat([jnp.where(sub[:8] < 4, last[:, 256 * g:256 * g + 128], last[:, 256 * g + 128:256 * g + 256])
                        for g in range(N2 // 8)], 0)
            nat = rep
            for e in range(1, 4):
                nat = jnp.where((sub & 3) == e, pltpu.roll(rep, 128 - N1 * e, 1), nat)
            wn[k] = nat

    da_chunk(0, spread([f for t, g in groups for f in radix_forward(t, g)], after_obuf, 24), filter_prep)

    def filt(p):
        out = [[], []]
        for k in range(2):
            v = [wq[k, t, pl.ds(pl.multiple_of(8 * p, 8), 8), :] for t in range(S // 128)]
            for e in range(2):
                out[e].append(_cat(unpack_pair(_cat([u[4 * e:4 * e + 4] for u in v], 0))))
        return out

    def beta_gu(w, j):
        quads = [wgu_v[w, 256 * half:256 * half + 256, 128 * (c + j):128 * (c + j + 1)].astype(F32)
                 for half in range(2) for c in (0, JH)]
        for k, v in enumerate(_beta(*quads)):
            bgu[w, k, j] = v.astype(BF)

    def spec_fwd_step(i, carry):
        for pp in range(UN // 2 + 1):
            if pp < UN // 2:
                for e in range(2):
                    spec = s_forward(i * UN + 2 * pp + e)
                    xs[i * UN + 2 * pp + e] = spec
            if pp > 0:
                for e, (wr, wi) in enumerate(filt(i * (UN // 2) + pp - 1)):
                    a = i * UN + 2 * (pp - 1) + e
                    xr, xi = xs[a, 0:N2, :], xs[a, N2:2 * N2, :]
                    s_inverse(a, xr * wr - xi * wi, xr * wi + xi * wr)
        return carry

    for cp in (wm_copy(2), wm_copy(3), wm_copy(4), do_copy(2), do_copy(3)):
        cp.start()
    jax.lax.fori_loop(0, N1 // UN, spec_fwd_step, 0)
    xr, xi = nyq_forward()
    xn[0], xn[1] = xr, xi
    nyq_inverse((xr * wn[0] - xi * wn[1]) * (1.0 / (S * D)), (xr * wn[1] + xi * wn[0]) * (1.0 / (S * D)))

    for cp in (do_copy(1), wm_copy(2), wm_copy(3), wm_copy(4)):
        cp.wait()
    radix = spread([f for t, g in groups for f in radix_inverse(t, g)], after_vbuf, 24)
    mods = spread([functools.partial(mod_block, b) for b in (2, 3, 4)], lambda v: after(scol, (5,), v), 24)
    da_chunk(1, lambda k, val: (radix(k, val), mods(k, val)))

    def y1_rows(i, part):
        for h in range(2):
            r0 = pl.multiple_of(2 * H * i + H * h + Q * part, Q)
            y1_v[pl.ds(r0, Q), :] = d_inverse(r0, Q, (2 * H * i + H * h + Q * part) // N2, 3)

    def ln2_rows(i, r):
        quads = []
        for h in range(2):
            rows = pl.ds(pl.multiple_of(2 * H * i + H * h + r, R), R)
            x1 = x_v[rows, :].astype(F32) + mod_row(2) * y1_v[rows, :]
            mu = _rowsum(_tiles(x1)) * (1.0 / D)
            xc = x1 - mu
            rstd = jax.lax.rsqrt(_rowsum(_tiles(xc * xc)) * (1.0 / D) + EPS)
            st2[0, rows, :] = jnp.broadcast_to(mu, (R, 128))
            st2[1, rows, :] = jnp.broadcast_to(rstd, (R, 128))
            h2 = (xc * rstd) * (1.0 + mod_row(4)) + mod_row(3)
            quads += [h2[:, :256], h2[:, 256:]]
        for k, v in enumerate(_alpha(*quads)):
            for t, tile in enumerate(_tiles(v)):
                ah[i, k, t, r:r + R, :] = tile.astype(BF)

    def ln2_step(n, carry):
        norms = spread([functools.partial(ln2_rows, 2 * n + m, r) for m in range(2) for r in range(0, H, R)],
                       lambda v: after(y1_v, (1,), v), 24)

        def between(k, val):
            norms(k, val)
            if k in (2, 8, 14):
                y1_rows(2 * n + (k + 4) // 12, (k // 6 + 1) % 2)

        do_copy(2 + n).wait()
        y1_rows(2 * n, 0)
        da_chunk(2 + n, between)
        return carry

    jax.lax.fori_loop(0, 2, ln2_step, 0)

    def row_out(src, dst, base, i):
        rows = pl.ds(pl.multiple_of(2 * H * i, 2 * H), 2 * H)
        return pltpu.make_async_copy(src.at[rows], dst.at[rows], osem.at[base + i])

    def gate_step(i, carry, first=False):
        halves = [half_rows(i, h) for h in range(2)]
        for j in range(JH):
            m = []
            for k in range(7):
                m.append(_dot(_bf(_cat([ah32[i, k, 0], ah32[i, k, 1]])), _bf(_cat([bgu32[0, k, j], bgu32[1, k, j]]))))
                if first and k < 2 and j + 1 < JH:
                    after(wgu_v, (0, 5), m[k])
                    beta_gu(k, j + 1)
            for q, gu in enumerate(_gamma_t(m)):
                jj, rows = JH * (q % 2) + j, halves[q // 2][1]
                res = _geglu(gu[:, :128], gu[:, 128:], da_v[jj, rows, :].astype(F32))
                for w in range(3):
                    act[w, jj, rows, :] = res[w].astype(BF)
        return carry

    for cp in wgu_copies:
        cp.wait()
    beta_gu(0, 0)
    beta_gu(1, 0)
    gate_step(0, 0, first=True)
    jax.lax.fori_loop(1, NTILE, gate_step, 0)

    def ffn_step(i, carry):
        halves = [half_rows(i, h) for h in range(2)]
        blocks = [[(JH * (q % 2) + j, halves[q // 2][0]) for j in range(JH)] for q in range(4)]
        for part in range(2):
            rows = [pl.ds(pl.multiple_of(2 * H * i + H * h + Q * part, Q), Q) for h in range(2)]
            dt, db = (do_v[r, :].astype(F32) * mod_row(5) for r in rows)
            for k, v in enumerate(_alpha(dt[:, :256], dt[:, 256:], db[:, :256], db[:, 256:])):
                lt[1, k, 2 * i + part] = v.astype(BF).T
                for t in range(2):
                    lt[0, k, 2 * i + part, 128 * t:128 * t + 128, :] = ah[i, k, t, Q * part:Q * part + Q, :].T
        cg, cu = operands(_gamma, 0, blocks, 1), operands(_gamma, 1, blocks, 1)
        ca = operands(_alpha, 2, blocks, 1)

        def ln2_bwd_rows(part, val):
            for r in range(0, Q, R):
                after(dx1_v, (1,), val[2 * r:2 * r + 8])
                rows = pl.ds(pl.multiple_of(2 * H * i + Q * part + r, R), R)
                y1 = y1_v[rows, :]
                dh2 = dx1_v[rows, :]
                rstd = _cat([st2[1, rows, :]] * 4)
                xhat = (x_v[rows, :].astype(F32) + mod_row(2) * y1 - _cat([st2[0, rows, :]] * 4)) * rstd
                dhx = dh2 * xhat
                sums[3] += _colsum8(dh2)
                sums[4] += _colsum8(dhx)
                cb1 = 1.0 + mod_row(4)
                dn = dh2 * cb1
                m1 = _rowsum(_tiles(dn)) * (1.0 / D)
                m2 = _rowsum(_tiles(dhx * cb1)) * (1.0 / D)
                dx1 = do_v[rows, :].astype(F32) + rstd * (dn - m1 - xhat * m2)
                dx1_v[rows, :] = dx1
                sums[2] += _colsum8(dx1 * y1)
            r0 = pl.multiple_of(2 * H * i + Q * part, Q)
            return lambda: d_forward(dx1_v[pl.ds(r0, Q), :] * mod_row(2), r0, (2 * H * i + Q * part) // N2, 1)

        dh, todo = {}, []
        for k in (5, 6, 0, 2, 4, 1, 3):
            pg = _dot_nt(cg[k], _bf(_cat([bgu32[0, k, j] for j in range(JH)])))
            if k in (1, 3):
                todo.append(ln2_bwd_rows(k // 2, pg))
            dh[k] = pg + _dot_nt(cu[k], _bf(_cat([bgu32[1, k, j] for j in range(JH)])))
            if k == 4:
                dx1_v[halves[0][1], :] = _cat([dh[0] + dh[2] + dh[4] - dh[5], dh[4] + dh[6]])
            if k == 3:
                dx1_v[halves[1][1], :] = _cat([dh[1] + dh[5], dh[0] + dh[1] + dh[3] - dh[6]])
                todo.pop(0)()
        y2 = {}
        for n, k in enumerate((1, 3, 2, 4, 0, 5, 6)):
            y2[k] = _dot(ca[k], _bf(_cat([bd32[k, 0], bd32[k, 1]])))
            if n in (0, 2):
                todo.append(ln2_bwd_rows(2 + n // 2, y2[k]))
            if n in (1, 3, 5):
                todo.pop(0)()
        for q, yv in enumerate(_gamma_t(y2)):
            rows, cols = halves[q // 2][1], slice(256 * (q % 2), 256 * (q % 2) + 256)
            sums[5, :, cols] += _colsum8(do_v[rows, cols].astype(F32) * yv)
            x1 = x_v[rows, cols].astype(F32) + mod_row(2)[:, cols] * y1_v[rows, cols]
            out_v[rows, cols] = (x1 + mod_row(5)[:, cols] * yv).astype(BF)
        row_out(out_v, out_hbm, 0, i).start()
        return carry

    jax.lax.fori_loop(0, NTILE, ffn_step, 0)

    def radix_fwd_step(t, carry):
        radix = spread([f for g in range(N2 // 8) for f in radix_forward(t, g)], after_obuf, 13)
        for n in range(2):
            dwgu_chunk(2 * t + n, shifted(radix, n))
        return carry

    jax.lax.fori_loop(0, 2, radix_fwd_step, 0)

    def spec_bwd_step(i, carry):
        def pair(pp):
            p = 4 * i + pp
            packed, out = [[], []], []
            for e, (wr, wi) in enumerate(filt(p)):
                a = 2 * p + e
                spec = s_forward(a)
                gr, gi = spec[:N2], spec[N2:]
                xr, xi = xs[a, 0:N2, :], xs[a, N2:2 * N2, :]
                for k, v in enumerate((gr * xr + gi * xi, gi * xr - gr * xi)):
                    packed[k].append(pltpu.bitcast(pltpu.pack_elementwise(_tiles(v), packed_dtype=BF), U32))
                out.append((a, gr * wr + gi * wi, gi * wr - gr * wi))
            for k in range(2):
                for t in range(S // 128):
                    dwq[k, t, pl.ds(pl.multiple_of(8 * p, 8), 8), :] = _cat([v[4 * t:4 * t + 4] for v in packed[k]], 0)
            return out

        pending = pair(0)

        def between(k, val):
            if k in (0, 2, 4):
                pending.extend(pair(k // 2 + 1))
            s_inverse(*pending.pop(0))

        dwgu_chunk(4 + i, between)
        s_inverse(*pending.pop(0))
        return carry

    jax.lax.fori_loop(0, 4, spec_bwd_step, 0)
    gr, gi = nyq_forward()
    gr, gi = gr * (1.0 / (S * D)), gi * (1.0 / (S * D))
    nyq_inverse(gr * wn[0] + gi * wn[1], gi * wn[0] - gr * wn[1])
    dwn = [gr * xn[0] + gi * xn[1], gi * xn[0] - gr * xn[1]]
    dwri_copies = [pltpu.make_async_copy(wri_v.at[k], dst, osem.at[10 + k]) for k, dst in enumerate((dwr_hbm, dwi_hbm))]
    for k in range(2):
        own = jnp.where(lane < N1, dwn[k], 0.0)
        flat = own
        for e in range(1, 4):
            flat = jnp.where((sub & 3) == e, pltpu.roll(own, N1 * e, 1), flat)
        pieces = []
        for g in range(N2 // 8):
            blk = flat[8 * g:8 * g + 8]
            pieces += [jnp.sum(jnp.where((sub[:8] < 4) == first, blk, 0.0), axis=0, keepdims=True) for first in (True, False)]
        wri_v[k, 256:257, :] = _cat(pieces).astype(BF)

    def radix_inv_step(t, carry):
        radix = spread([f for g in range(N2 // 8) for f in radix_inverse(t, g)], after_vbuf, 13)
        for n in range(2):
            dwgu_chunk(8 + 2 * t + n, shifted(radix, n))
        for u in range(S // 128):
            wri_v[t, 0:256, 128 * u:128 * u + 128] = _bf(jnp.take_along_axis(
                dwq[t, u].T, 4 * (lane_d & (N1 - 1)) + (lane_d >> 5), axis=1))
        return carry

    jax.lax.fori_loop(0, 2, radix_inv_step, 0)
    for cp in dwri_copies:
        cp.start()

    def dh1_rows(i, part):
        r0 = pl.multiple_of(2 * H * i + Q * part, Q)
        y1_v[pl.ds(r0, Q), :] = d_inverse(r0, Q, (2 * H * i + Q * part) // N2, 2)

    def ln1_bwd_rows(i, r):
        rows = pl.ds(pl.multiple_of(2 * H * i + r, R), R)
        dh1 = y1_v[rows, :]
        rstd = _cat([st1[1, rows, :]] * 4)
        xhat = (x_v[rows, :].astype(F32) - _cat([st1[0, rows, :]] * 4)) * rstd
        dhx = dh1 * xhat
        sums[0] += _colsum8(dh1)
        sums[1] += _colsum8(dhx)
        ca1 = 1.0 + mod_row(1)
        dn = dh1 * ca1
        m1 = _rowsum(_tiles(dn)) * (1.0 / D)
        m2 = _rowsum(_tiles(dhx * ca1)) * (1.0 / D)
        dx_v[rows, :] = (dx1_v[rows, :] + rstd * (dn - m1 - xhat * m2)).astype(BF)

    def ln1_bwd_step(i, carry):
        norms = spread([functools.partial(ln1_bwd_rows, i, r) for r in range(0, 2 * H, R)],
                       lambda v: after(y1_v, (1,), v), 6)

        def between(k, val):
            norms(k, val)
            if k in (0, 1, 3):
                dh1_rows(i, (k + 3) // 2)

        dh1_rows(i, 0)
        dwd_chunk(i, between)
        dwd_start(i)
        row_out(dx_v, dx_hbm, 4, i).start()
        return carry

    jax.lax.fori_loop(0, NTILE, ln1_bwd_step, 0)
    dcacc[...] = jnp.zeros(dcacc.shape, F32)

    def dwm_copy(b, t):
        cols = pl.ds(pl.multiple_of(D * b + 128 * t, 128), 128)
        return pltpu.make_async_copy(dwm_v.at[b, t], dwm_hbm.at[:, cols], osem.at[12])

    def mod_grad(b, r):
        dmod = jnp.sum(sums[b], axis=0, keepdims=True).astype(BF).astype(F32)
        sc = scol[r:r + Q, :]
        for t, tile in enumerate(_tiles(dmod)):
            dwm_v[b, t, r:r + Q, :] = (sc * tile).astype(BF)
        prod = _tiles(wm_v[b, r:r + Q, :].astype(F32) * dmod)
        dcacc[r:r + Q, :] += (prod[0] + prod[1]) + (prod[2] + prod[3])

    def mod_grad_step(n, carry):
        work = [functools.partial(mod_grad, 3 * n + b, r) for b in range(3) for r in range(0, D, Q)]
        dwgu_chunk(12 + n, spread(work, lambda v: after(sums, (4, 0), v), 6))
        for b in range(3):
            for t in range(4):
                dwm_copy(3 * n + b, t).start()
        return carry

    jax.lax.fori_loop(0, 2, mod_grad_step, 0)
    ds = jnp.sum(dcacc[...].T, axis=0, keepdims=True).astype(BF).astype(F32)
    dc_ref[...] = (ds * (sig * (1.0 + cv * (1.0 - sig)))).astype(BF)
    for cp in dwgu_copies:
        cp.start()

    def dwd_step(j, carry):
        dwd_chunk(j, lambda k, val: None)
        dwd_start(j)
        return carry

    jax.lax.fori_loop(NTILE, JH, dwd_step, 0)

    for i in range(NTILE):
        row_out(out_v, out_hbm, 0, i).wait()
        row_out(dx_v, dx_hbm, 4, i).wait()
    for cp in dwri_copies + dwgu_copies:
        cp.wait()
    for b in range(6):
        for t in range(4):
            dwm_copy(b, t).wait()
    for j in range(JH):
        for half in range(2):
            dwd_copy(j, half).wait()


@jax.jit
def pallas_adaLN_cond__spectral_gfnet__geglu_ffn__prompt_kernel(
    A_x: jax.Array,
    A_w_r: jax.Array,
    A_w_i: jax.Array,
    B_x: jax.Array,
    B_w_gate: jax.Array,
    B_w_up: jax.Array,
    B_w_down: jax.Array,
    c: jax.Array,
    w_mod: jax.Array,
    grad_out: jax.Array,
):
    del B_x
    vm = pltpu.VMEM
    hbm = pl.BlockSpec(memory_space=pl.ANY)
    sds = jax.ShapeDtypeStruct
    scratch = [
        vm((S + 64, D), BF), vm((S, D), BF), vm((2, D // 2 + 1, S), BF), vm((2, D + 64, F), BF),
        vm((F, D), BF), vm((6, D, D), BF), vm((8, 128, 128), BF), vm((N1, 128, 128), BF),
        vm((4, 6, 128, 128), BF), vm((N1, 128, 128), BF), vm((D + 128, 128), F32), vm((8, 8, D), F32),
        vm((2, 7, JH, 256, 128), BF), vm((7, 2, F // 2, 128), BF),
        vm((4, S + 128, 128), F32), vm((2, N1, 128, 128), BF), vm((2, N1 + 1, 128, 128), F32),
        vm((N1, 128, 256), F32), vm((2, S // 128, 128, 128), U32), vm((2, S // 128, 128, 128), U32),
        vm((2, N2, 128), F32), vm((2, N2, 128), F32), vm((N2, 128), F32),
        vm((S + 32, D), F32), vm((2, S, 128), F32), vm((2, S, 128), F32),
        vm((NTILE, 7, 2, H, 128), BF), vm((2, 7, 2 * NTILE, 256, 128), BF), vm((3, 2 * JH, S, 128), BF),
        vm((2 * JH, S, 128), BF), vm((S, D), BF), vm((S, D), BF), vm((S + 32, D), F32), vm((6, 4, D, 128), BF),
        vm((8, 8, D), F32), vm((D, 128), F32),
        pltpu.SemaphoreType.DMA((24,)), pltpu.SemaphoreType.DMA((14,)),
    ]
    outs = pl.pallas_call(
        _kernel,
        in_specs=[pl.BlockSpec(memory_space=pltpu.SMEM)] + [pl.BlockSpec(memory_space=vm)] * 2 + [hbm] * 10,
        out_specs=[hbm] * 7 + [pl.BlockSpec(memory_space=vm), hbm],
        out_shape=[sds((S, D), BF), sds((S, D), BF), sds((D // 2 + 1, S), BF), sds((D // 2 + 1, S), BF), sds((D, F), BF),
                   sds((D, F), BF), sds((F, D), BF), sds((1, D), BF), sds((D, 6 * D), BF)],
        scratch_shapes=scratch,
        compiler_params=pltpu.CompilerParams(vmem_limit_bytes=124 * 2 ** 20),
    )(_SPARE, c, _TWID, A_x.reshape(S, D), grad_out.reshape(S, D), A_w_r.T, A_w_i.T, B_w_gate, B_w_up, B_w_down, w_mod, _DMAT, _MF)
    return (outs[0].reshape(1, S, D), outs[1].reshape(1, S, D), outs[2].T, outs[3].T) + tuple(outs[4:])
```

```python
import functools
import math

import numpy as np
import jax
import jax.numpy as jnp
import jax.experimental.pallas as pl
import jax.experimental.pallas.tpu as pltpu

S, D, F = 2048, 512, 1792
N1, N2 = 32, 64
H = 256
NTILE = S // (2 * H)
Q = 128
R = 16
JH = F // 256
BF, F32, U32 = jnp.bfloat16, jnp.float32, jnp.uint32
EPS = 1e-5
G0 = math.sqrt(2.0 / math.pi)
G1 = 0.044715 * G0


def _constants():
    r = np.arange(128)[:, None].astype(np.float64)
    l = np.arange(128)[None, :]
    ev = l % 2 == 0
    th = lambda k: 2.0 * np.pi * k * r / D
    k_im = 2.0 * ((l - 1) % 128)
    d0 = np.where(ev, np.cos(th(2.0 * l)), -np.sin(th(k_im)))
    d2 = np.where(ev, -np.sin(th(k_im)), np.cos(th(2.0 * l)))
    odd = th(2.0 * l + 1.0)
    p_re, p_im = np.cos(odd), -np.sin(odd)
    q_re = np.where(ev, -np.sin(odd), np.sin(odd))
    q_im = np.where(ev, -np.cos(odd), np.cos(odd))
    dmat = np.stack([d0, d2, p_re, q_re, p_im, q_im])
    weave = lambda re, im: np.stack([v.reshape(-1, N2 // 8, 8) for v in (re, im)], axis=2).reshape(-1, 2 * N2)
    phi = 2.0 * np.pi * ((np.arange(N2)[:, None] * np.arange(N2)[None, :]) % N2) / N2
    c, s = np.cos(phi), np.sin(phi)
    base = weave(np.concatenate([c, -s]), np.concatenate([s, c]))
    turn = weave(np.concatenate([-s, -c]), np.concatenate([c, -s]))
    theta = 2.0 * np.pi * np.arange(N1)[:, None] * np.arange(N2)[None, :] / S
    mf = np.concatenate([base, turn, weave(np.cos(theta), np.cos(theta)), weave(np.sin(theta), np.sin(theta))])
    a = np.arange(128)[:, None]
    ok = (a < N1) & (l < N1)
    fc = np.where(ok, np.cos(2.0 * np.pi * ((a * l) % N1) / N1), 0.0)
    fs = np.where(ok, -np.sin(2.0 * np.pi * ((a * l) % N1) / N1), 0.0)
    tw = 2.0 * np.pi * np.arange(N2)[:, None] * l / S
    twid = np.stack([np.cos(tw), np.sin(tw)]).astype(np.float32)
    dmat = np.concatenate([dmat, fc[None], fs[None]]).astype(np.float32).astype(jnp.bfloat16)
    return dmat, mf.astype(np.float32), twid


_DMAT, _MF, _TWID = _constants()
_SPARE = np.array([0, S, N1, 2 * JH, 6, D, 0, S // 128], np.int32)


def _dot(a, b):
    return jax.lax.dot_general(a, b, (((1,), (0,)), ((), ())), preferred_element_type=F32)


def _dot_nt(a, b):
    return jax.lax.dot_general(a, b, (((1,), (1,)), ((), ())), preferred_element_type=F32)


def _cat(xs, axis=1):
    return jnp.concatenate(xs, axis=axis)


def _tiles(v):
    return [v[:, 128 * t:128 * t + 128] for t in range(v.shape[1] // 128)]


def _alpha(a11, a12, a21, a22):
    return [a11 + a22, a21 + a22, a11, a22, a11 + a12, a21 - a11, a12 - a22]


def _beta(b11, b12, b21, b22):
    return [b11 + b22, b11, b12 - b22, b21 - b11, b22, b11 + b12, b21 + b22]


def _gamma(c11, c12, c21, c22):
    return [c11 + c22, c21 - c22, c12 + c22, c11 + c21, c12 - c11, c22, c11]


def _alpha_t(p):
    return [p[0] + p[2] + p[4] - p[5], p[4] + p[6], p[1] + p[5], p[0] + p[1] + p[3] - p[6]]


def _beta_t(q):
    return [q[0] + q[1] - q[3] + q[5], q[2] + q[5], q[3] + q[6], q[0] - q[2] + q[4] + q[6]]


def _gamma_t(m):
    return [m[0] + m[3] - m[4] + m[6], m[2] + m[4], m[1] + m[3], m[0] - m[1] + m[2] + m[5]]


_PLAIN = {_alpha: {2: 0, 3: 3}, _gamma: {5: 3, 6: 0}}


def aligned(v, n):
    return v if isinstance(v, int) else pl.multiple_of(v, n)


def _bf(words):
    return pltpu.bitcast(words, BF)


def _twiddle(z, k, n, sign):
    re, im = z
    k %= n
    if k == 0:
        return z
    if 8 * k == n or 8 * k == 3 * n:
        h = math.sqrt(0.5)
        if 8 * k == n:
            return ((re - im) * h, (re + im) * h) if sign > 0 else ((re + im) * h, (im - re) * h)
        return ((re + im) * (-h), (re - im) * h) if sign > 0 else ((im - re) * h, (re + im) * (-h))
    c, s = math.cos(2.0 * math.pi * k / n), sign * math.sin(2.0 * math.pi * k / n)
    return (re * c - im * s, re * s + im * c)


def _dft(z, sign):
    n = len(z)
    if n == 1:
        return z
    if n == 2:
        return [(z[0][0] + z[1][0], z[0][1] + z[1][1]), (z[0][0] - z[1][0], z[0][1] - z[1][1])]
    u, v, w = _dft(z[0::2], sign), _dft(z[1::4], sign), _dft(z[3::4], sign)
    out = [None] * n
    q = n // 4
    for k in range(q):
        a, b = _twiddle(v[k], k, n, sign), _twiddle(w[k], 3 * k, n, sign)
        sr, si = a[0] + b[0], a[1] + b[1]
        dr, di = a[0] - b[0], a[1] - b[1]
        out[k] = (u[k][0] + sr, u[k][1] + si)
        out[k + 2 * q] = (u[k][0] - sr, u[k][1] - si)
        plus = (u[k + q][0] - di, u[k + q][1] + dr)
        minus = (u[k + q][0] + di, u[k + q][1] - dr)
        out[k + q], out[k + 3 * q] = (plus, minus) if sign > 0 else (minus, plus)
    return out


def _rowsum(tiles):
    acc = tiles[0]
    for t in tiles[1:]:
        acc = acc + t
    return jnp.sum(acc, axis=1, keepdims=True)


def _colsum8(v):
    parts = [v[r:r + 8] for r in range(0, v.shape[0], 8)]
    while len(parts) > 1:
        parts = [parts[i] + parts[i + 1] for i in range(0, len(parts), 2)]
    return parts[0]


def _geglu(g, u, da):
    g2 = g * g
    cdf = 0.5 * jnp.tanh(g * (G0 + G1 * g2)) + 0.5
    ge = g * cdf
    dge = cdf + (ge * (1.0 - cdf)) * (2.0 * G0 + (6.0 * G1) * g2)
    return da * (u * dge), da * ge, ge * u


def _kernel(spare_hbm, c_hbm, twid_hbm, x_hbm, do_hbm, wr_hbm, wi_hbm, wg_hbm, wu_hbm, wd_hbm, wm_hbm, dmat_hbm, mf_hbm,
            out_hbm, dx_hbm, dwr_hbm, dwi_hbm, dwg_hbm, dwu_hbm, dwd_hbm, dc_ref, dwm_hbm,
            x_v, do_v, wri_v, wgu_v, wd_v, wm_v, dmat_v, mf_v,
            dall, mi_v, scol, mod_v, bgu, bd, obuf, zbuf, vbuf, xs, wq, dwq, wn, xn, nyq,
            y1_v, st1, st2, ah, lt, act, da_v, out_v, dx_v, dx1_v, dwm_v, sums, dcacc, spare_ref, c_ref, twid_ref, gen_ref, isem, osem):
    lane = jax.lax.broadcasted_iota(jnp.int32, (N2, 128), 1)
    lane_h = jax.lax.broadcasted_iota(jnp.int32, (H, 128), 1)
    even_h = (lane_h & 1) == 0
    sgn_h = (1 - 2 * (lane_h & 1)).astype(F32)

    dall32, bgu32, bd32, zbuf32, ah32, lt32, act32, da32 = (
        r.bitcast(U32) for r in (dall, bgu, bd, zbuf, ah, lt, act, da_v))

    def wm_copy(b):
        return pltpu.make_async_copy(wm_hbm.at[:, pl.ds(D * b, D)], wm_v.at[b], isem.at[b])

    def row_copy(src, dst, base, i):
        rows = pl.ds(2 * H * i, 2 * H)
        return pltpu.make_async_copy(src.at[rows], dst.at[rows], isem.at[base + i])

    x_copy = lambda i: row_copy(x_hbm, x_v, 6, i)
    do_copy = lambda i: row_copy(do_hbm, do_v, 10, i)
    col_groups = [(j, min(j + 2, JH)) for j in range(0, JH, 2)]


    wd_copy = pltpu.make_async_copy(wd_hbm, wd_v, isem.at[20])
    small_copies = [pltpu.make_async_copy(src, dst, isem.at[21 + k]) for k, (src, dst) in
                    enumerate(((c_hbm, c_ref), (spare_hbm, spare_ref), (twid_hbm, twid_ref), (mf_hbm, gen_ref)))]
    wgu_copies = [pltpu.make_async_copy(src, wgu_v.at[w, pl.ds(0, D)], isem.at[14 + w])
                  for w, src in enumerate((wg_hbm, wu_hbm))]
    dmat_copy = pltpu.make_async_copy(dmat_hbm, dmat_v, isem.at[16])
    wri_copies = [pltpu.make_async_copy(src, wri_v.at[k], isem.at[18 + k]) for k, src in enumerate((wr_hbm, wi_hbm))]

    for cp in small_copies + [wm_copy(0), wm_copy(1), dmat_copy, x_copy(0), x_copy(1)]:
        cp.start()
    for cp in small_copies:
        cp.wait()

    for a in range(N1):
        m = (gen_ref[0:128, :] * gen_ref[256 + a:257 + a, :] + gen_ref[128:256, :] * gen_ref[256 + N1 + a:257 + N1 + a, :])
        mf_v[a] = m.astype(BF)
        mi_v[a] = m.T.astype(BF)

    cv = c_ref[...].astype(F32)
    sig = 1.0 / (1.0 + jnp.exp(-cv))
    s_row = (cv * sig).astype(BF).astype(F32)
    scol[0:D, :] = jnp.broadcast_to(s_row, (128, D)).T

    def mod_block(b):
        sc = scol[0:D, :]
        parts = [_colsum8(t.astype(F32) * sc) for t in _tiles(wm_v[b])]
        tot = jnp.sum(_cat(parts), axis=0, keepdims=True)
        mod_v[b] = jnp.broadcast_to(tot.astype(BF).astype(F32), (8, D))

    def mod_row(b):
        return mod_v[b, 0:1, :]

    sums[...] = jnp.zeros(sums.shape, F32)
    nyq[...] = jnp.zeros(nyq.shape, F32)
    wm_copy(0).wait()
    for cp in (x_copy(2), x_copy(3)):
        cp.start()
    mod_block(0)
    wm_copy(1).wait()
    mod_block(1)

    dmat_copy.wait()
    lane_d = jax.lax.broadcasted_iota(jnp.int32, (128, 128), 1)
    for k in range(6):
        m = dmat_v[k]
        scale = jnp.where(lane_d == 0, 1.0 / (S * D), 2.0 / (S * D)) if k == 0 else 2.0 / (S * D)
        ms = m.astype(F32) * scale
        dall[0, k] = m
        dall[1, k] = ms.astype(BF)
        dall[2, k] = m.astype(F32).T.astype(BF)
        dall[3, k] = ms.T.astype(BF)

    def after(ref, lead, val):
        rows = 8 * 4 // ref.dtype.itemsize
        idx = tuple(spare_ref[k] for k in lead[:-1]) + (pl.ds(pl.multiple_of(spare_ref[lead[-1]], rows), rows),)
        ref[idx + (slice(0, 128),)] = val[0:rows, 0:128].astype(ref.dtype)

    def d_forward(h, r0, a0, sel):
        n = h.shape[0]
        h0, h1, h2, h3 = _tiles(h)
        t0, t1 = h0 + h2, h1 + h3
        z0, z2 = t0 + t1, t0 - t1
        o0 = _dot(z0.astype(BF), dall[sel, 0])
        o2 = _dot(z2.astype(BF), dall[sel, 1])
        dd = _bf(_cat([_cat([dall32[sel, 2], dall32[sel, 3]], 0), _cat([dall32[sel, 4], dall32[sel, 5]], 0)]))
        odd = _dot(_cat([h0 - h2, h1 - h3]).astype(BF), dd)
        rows = pl.ds(r0, n)
        obuf[0, rows, :] = jnp.where(even_h[:n], o0, o2)
        obuf[1, rows, :] = odd[:, :128]
        obuf[2, rows, :] = pltpu.roll(jnp.where(even_h[:n], o2, o0), 127, 1)
        obuf[3, rows, :] = odd[:, 128:]
        ncol = jnp.sum(z0 * sgn_h[:n], axis=1, keepdims=True)
        acc = nyq[...]
        for t in range(n // N2):
            acc = jnp.where(lane == a0 + t, ncol[N2 * t:N2 * t + N2], acc)
        nyq[...] = acc

    def d_inverse(r0, n, a0, sel):
        rows = pl.ds(r0, n)
        re_e, im_e = obuf[0, rows, :], pltpu.roll(obuf[2, rows, :], 1, 1)
        z0 = _dot(jnp.where(even_h[:n], re_e, im_e).astype(BF), dall[sel, 0])
        z2 = _dot(jnp.where(even_h[:n], im_e, re_e).astype(BF), dall[sel, 1])
        dd = _bf(_cat([_cat([dall32[sel, 2], dall32[sel, 4]], 0), _cat([dall32[sel, 3], dall32[sel, 5]], 0)]))
        pq = _dot(_cat([obuf[1, rows, :], obuf[3, rows, :]]).astype(BF), dd)
        nq = nyq[...]
        ncol = _cat([jnp.sum(jnp.where(lane == a0 + t, nq, 0.0), axis=1, keepdims=True) for t in range(n // N2)], 0)
        z0 = z0 + ncol * sgn_h[:n]
        t0, t1 = z0 + z2, z0 - z2
        p, q = pq[:, :128], pq[:, 128:]
        return _cat([t0 + p, t1 + q, t0 - p, t1 - q])

    def radix_steps(load, store, sign):
        z = [None] * N1

        def step(first):
            for a in range(first, N1, 4):
                z[a] = load(a)
            if first == 3:
                for a, (re, im) in enumerate(_dft(z, sign)):
                    store(a, re, im)

        return [functools.partial(step, first) for first in (0, 2, 1, 3)] + [None]

    def radix_forward(t, g):
        rows = lambda a: pl.ds(aligned(N2 * a + 8 * g, 8), 8)

        def store(a, re, im):
            zbuf[t, a, pl.ds(aligned(16 * g, 16), 16), :] = _cat([re, im], 0).astype(BF)

        return radix_steps(lambda a: (obuf[t, rows(a), :], obuf[2 + t, rows(a), :]), store, -1)

    def radix_inverse(t, g):
        def store(a, re, im):
            obuf[t, N2 * a + 8 * g:N2 * a + 8 * g + 8, :] = re
            obuf[2 + t, N2 * a + 8 * g:N2 * a + 8 * g + 8, :] = im

        return radix_steps(lambda a: (vbuf[t, a, 16 * g:16 * g + 8, :], vbuf[t, a, 16 * g + 8:16 * g + 16, :]), store, 1)

    after_obuf = lambda v: after(obuf, (0, 1), v)
    after_vbuf = lambda v: after(vbuf, (0, 2, 0), v)

    def interleave8(re, im):
        return _cat([v[8 * g:8 * g + 8] for g in range(N2 // 8) for v in (re, im)], 0)

    def nyquist(filter_fn):
        n = nyq[...].astype(BF)
        zr, zi = _dot(n, dmat_v[6]), _dot(n, dmat_v[7])
        yield
        tc, ts = twid_ref[0], twid_ref[1]
        xq = _dot(mf_v[0], interleave8(zr * tc + zi * ts, zi * tc - zr * ts).astype(BF))
        yield
        v = _dot(mi_v[0], _cat(filter_fn(xq[:N2], xq[N2:]), 0).astype(BF))
        yield
        vr = _cat([v[16 * g:16 * g + 8] for g in range(N2 // 8)], 0)
        vi = _cat([v[16 * g + 8:16 * g + 16] for g in range(N2 // 8)], 0)
        nyq[...] = (_dot((vr * tc - vi * ts).astype(BF), dmat_v[6]) + _dot((vr * ts + vi * tc).astype(BF), dmat_v[7]))

    def unpack_pair(w):
        return pltpu.bitcast(w << 16, F32), pltpu.bitcast(w & jnp.uint32(0xFFFF0000), F32)

    UN = 16

    def s_forward(a):
        return _dot(mf_v[a], _bf(_cat([zbuf32[0, a], zbuf32[1, a]])))

    def s_inverse(a, yr, yi):
        v = _dot(mi_v[a], _cat([yr, yi], 0).astype(BF))
        vbuf[0, a] = v[:, :128]
        vbuf[1, a] = v[:, 128:]

    def da_chunk(i, between, group_start=lambda n: None):
        top, bot = pl.ds(aligned(2 * H * i, H), H), pl.ds(aligned(2 * H * i + H, H), H)
        gb = mod_row(5)
        dt, db = do_v[top, :].astype(F32) * gb, do_v[bot, :].astype(F32) * gb
        quads = [dt[:, :256], dt[:, 256:], db[:, :256], db[:, 256:]]
        lhs = [g.astype(BF) for g in _gamma(*quads)]
        for n, (j0, j1) in enumerate(col_groups):
            words = slice(64 * j0, 64 * j1)
            group_start(n)
            p = {}
            for step, k in enumerate((1, 5, 0, 2, 4, 6, 3)):
                p[k] = _dot_nt(lhs[k], _bf(_cat([bd32[k, 0, words, :], bd32[k, 1, words, :]])))
                between(7 * n + step, p[k])
            p = _alpha_t(p)
            for q in (2, 0, 1, 3):
                for j, tile in enumerate(_tiles(p[q])):
                    da_v[JH * (q % 2) + j0 + j, top if q < 2 else bot, :] = tile.astype(BF)

    def operands(fn, w, blocks, axis):
        sums_f32 = fn(*[_cat([act[w, j, pl.ds(r, H), :].astype(F32) for j, r in blk], axis) for blk in blocks])
        out = []
        for k in range(7):
            if k in _PLAIN[fn]:
                half = lambda r: aligned(r // 2, H // 2)
                out.append(_bf(_cat([act32[w, j, pl.ds(half(r), H // 2), :] for j, r in blocks[_PLAIN[fn][k]]], axis)))
            else:
                out.append(sums_f32[k].astype(BF))
        return out

    def dw_blocks(w, j, between):
        blocks = [[(JH * (q % 2) + j, 2 * H * i + H * (q // 2)) for i in range(NTILE)] for q in range(4)]
        q, rhs = {}, operands(_gamma, w, blocks, 0)
        for step, k in enumerate((5, 6, 2, 3, 0, 1, 4)):
            q[k] = _dot(_bf(_cat([lt32[w // 2, k, t] for t in range(2 * NTILE)])), rhs[k])
            between(step, q[k])
        q = _beta_t(q)
        return [(n, q[n]) for n in (1, 2, 0, 3)]

    dwgu_copies = [pltpu.make_async_copy(wgu_v.at[w, pl.ds(0, D)], dst, osem.at[8 + w])
                   for w, dst in enumerate((dwg_hbm, dwu_hbm))]

    def dwgu_chunk(n, between):
        w, j = n // JH, n % JH
        for q, blk in dw_blocks(w, j, between):
            cols = pl.ds(aligned(128 * (JH * (q % 2) + j), 128), 128)
            wgu_v[w, 256 * (q // 2):256 * (q // 2) + 256, cols] = blk.astype(BF)

    def dwd_copy(j, half):
        rows = pl.ds(aligned((F // 2) * half + 128 * j, 128), 128)
        return pltpu.make_async_copy(wd_v.at[rows], dwd_hbm.at[rows], osem.at[13])

    def dwd_chunk(j, between):
        for q, blk in dw_blocks(2, j, between):
            rows = pl.ds(aligned((F // 2) * (q % 2) + 128 * j, 128), 128)
            wd_v[rows, 256 * (q // 2):256 * (q // 2) + 256] = blk.T.astype(BF)

    def dwd_start(j):
        for half in range(2):
            dwd_copy(j, half).start()

    def shifted(between, n):
        return lambda k, val: between(7 * n + k, val)

    def half_rows(i, h):
        r0 = aligned(2 * H * i + H * h, H)
        return r0, pl.ds(r0, H), (2 * H * i + H * h) // N2

    def spread(work, tie, slots):
        def between(k, val):
            todo = work[k * len(work) // slots:(k + 1) * len(work) // slots]
            for n, thunk in enumerate(todo):
                if thunk is not None:
                    r = (n * val.shape[0] // len(todo)) // 16 * 16
                    tie(val[r:r + 16])
                    thunk()
        return between

    def ln1_step(i, carry):
        x_copy(i).wait()

        @pl.when(i == 1)
        def _():
            for cp in (wm_copy(5), do_copy(0), wd_copy):
                cp.start()

        @pl.when(i == NTILE - 1)
        def _():
            for cp in wri_copies:
                cp.start()

        for part in range(2 * H // Q):
            r0 = pl.multiple_of(2 * H * i + Q * part, Q)
            rows = pl.ds(r0, Q)
            xv = x_v[rows, :].astype(F32)
            mu = _rowsum(_tiles(xv)) * (1.0 / D)
            xc = xv - mu
            rstd = jax.lax.rsqrt(_rowsum(_tiles(xc * xc)) * (1.0 / D) + EPS)
            st1[0, rows, :] = jnp.broadcast_to(mu, (Q, 128))
            st1[1, rows, :] = jnp.broadcast_to(rstd, (Q, 128))
            after(x_v, (1,), xc)
            d_forward((xc * rstd) * (1.0 + mod_row(1)) + mod_row(0), r0, (2 * H * i + Q * part) // N2, 0)
        return carry

    jax.lax.fori_loop(0, NTILE, ln1_step, 0, unroll=2)
    groups = [(t, g) for t in range(2) for g in range(N2 // 8)]

    def early_radix_step(g, carry):
        for t in range(2):
            for thunk in radix_forward(t, g)[:-1]:
                thunk()
        return carry

    jax.lax.fori_loop(0, N2 // 8, early_radix_step, 0)
    for cp in (wm_copy(5), do_copy(0), wd_copy):
        cp.wait()
    mod_block(5)

    def beta_d(n):
        j0, j1 = col_groups[n]
        for t in range(2):
            quads = [wd_v[pl.ds((F // 2) * half + 128 * j0, 128 * (j1 - j0)), 128 * (c + t):128 * (c + t + 1)].astype(F32)
                     for half in range(2) for c in (0, 2)]
            for k, v in enumerate(_beta(*quads)):
                bd[k, t, 128 * j0:128 * j1, :] = v.astype(BF)

    sub = jax.lax.broadcasted_iota(jnp.int32, (N2, 128), 0)

    def filter_prep(n):
        beta_d(n)
        if n != 2:
            return
        for cp in wri_copies:
            cp.wait()
        for cp in (do_copy(1), wm_copy(2), wm_copy(3), wm_copy(4)):
            cp.start()
        for k in range(2):
            for t in range(S // 128):
                words = pltpu.bitcast(wri_v[k, 0:256, 128 * t:128 * t + 128], U32)
                wq[k, t] = jnp.take_along_axis(words, (lane_d >> 2) + N1 * (lane_d & 3), axis=1).T
            last = wri_v[k, 256:257, :].astype(F32)
            rep = _cat([jnp.where(sub[:8] < 4, last[:, 256 * g:256 * g + 128], last[:, 256 * g + 128:256 * g + 256])
                        for g in range(N2 // 8)], 0)
            nat = rep
            for e in range(1, 4):
                nat = jnp.where((sub & 3) == e, pltpu.roll(rep, 128 - N1 * e, 1), nat)
            wn[k] = nat

    da_chunk(0, lambda k, val: None, filter_prep)

    def filt(p):
        out = [[], []]
        for k in range(2):
            v = [wq[k, t, pl.ds(pl.multiple_of(8 * p, 8), 8), :] for t in range(S // 128)]
            for e in range(2):
                out[e].append(_cat(unpack_pair(_cat([u[4 * e:4 * e + 4] for u in v], 0))))
        return out

    def beta_gu(w, j):
        quads = [wgu_v[w, 256 * half:256 * half + 256, 128 * (c + j):128 * (c + j + 1)].astype(F32)
                 for half in range(2) for c in (0, JH)]
        for k, v in enumerate(_beta(*quads)):
            bgu[w, k, j] = v.astype(BF)

    def spec_fwd_step(i, carry):
        for pp in range(UN // 2 + 1):
            if pp < UN // 2:
                for e in range(2):
                    spec = s_forward(i * UN + 2 * pp + e)
                    xs[i * UN + 2 * pp + e] = spec
            if pp > 0:
                for e, (wr, wi) in enumerate(filt(i * (UN // 2) + pp - 1)):
                    a = i * UN + 2 * (pp - 1) + e
                    xr, xi = xs[a, 0:N2, :], xs[a, N2:2 * N2, :]
                    s_inverse(a, xr * wr - xi * wi, xr * wi + xi * wr)
        return carry

    jax.lax.fori_loop(0, N1 // UN, spec_fwd_step, 0)

    def nyq_filter(xr, xi):
        xn[0], xn[1] = xr, xi
        return [(xr * wn[0] - xi * wn[1]) * (1.0 / (S * D)), (xr * wn[1] + xi * wn[0]) * (1.0 / (S * D))]

    side = nyquist(nyq_filter)
    for cp in (do_copy(1), wm_copy(2), wm_copy(3), wm_copy(4)):
        cp.wait()
    radix = spread([f for t, g in groups for f in radix_inverse(t, g)], after_vbuf, 24)
    mods = spread([functools.partial(mod_block, b) for b in (2, 3, 4)], lambda v: after(scol, (5,), v), 24)
    da_chunk(1, lambda k, val: (radix(k, val), mods(k, val), k % 2 and next(side, None)),
             lambda n: do_copy(n + 1).start() if n in (1, 2) else None)

    def y1_rows(i, part):
        for h in range(2):
            r0 = 2 * H * i + H * h + Q * part
            y1_v[pl.ds(r0, Q), :] = d_inverse(r0, Q, r0 // N2, 3)

    def ln2_rows(i, r):
        quads = []
        for h in range(2):
            rows = pl.ds(2 * H * i + H * h + r, R)
            x1 = x_v[rows, :].astype(F32) + mod_row(2) * y1_v[rows, :]
            mu = _rowsum(_tiles(x1)) * (1.0 / D)
            xc = x1 - mu
            rstd = jax.lax.rsqrt(_rowsum(_tiles(xc * xc)) * (1.0 / D) + EPS)
            st2[0, rows, :] = jnp.broadcast_to(mu, (R, 128))
            st2[1, rows, :] = jnp.broadcast_to(rstd, (R, 128))
            h2 = (xc * rstd) * (1.0 + mod_row(4)) + mod_row(3)
            quads += [h2[:, :256], h2[:, 256:]]
        for k, v in enumerate(_alpha(*quads)):
            for t, tile in enumerate(_tiles(v)):
                ah[i, k, t, r:r + R, :] = tile.astype(BF)

    norms = spread([functools.partial(ln2_rows, i, r) for i in range(NTILE) for r in range(0, H, R)],
                   lambda v: after(y1_v, (1,), v), 52)

    def ln2_between(k, val):
        norms(k, val)
        if k % 6 == 2 and k < 42:
            y1_rows(*divmod(k // 6 + 1, 2))

    for cp in wgu_copies:
        cp.start()
    for cp in (do_copy(2), do_copy(3)):
        cp.wait()
    y1_rows(0, 0)
    for n in range(2):
        da_chunk(2 + n, lambda k, val: ln2_between(28 * n + k, val))

    def row_out(src, dst, base, i):
        rows = pl.ds(aligned(2 * H * i, 2 * H), 2 * H)
        return [pltpu.make_async_copy(src.at[t, rows], dst.at[rows, pl.ds(128 * t, 128)], osem.at[base + i])
                for t in range(4)]

    def gate_step(i, carry, first=False):
        halves = [half_rows(i, h) for h in range(2)]
        for j in range(JH):
            m = []
            for k in range(7):
                m.append(_dot(_bf(_cat([ah32[i, k, 0], ah32[i, k, 1]])), _bf(_cat([bgu32[0, k, j], bgu32[1, k, j]]))))
                if first and k < 2 and j + 1 < JH:
                    after(wgu_v, (0, 5), m[k])
                    beta_gu(k, j + 1)
            quads = _gamma_t(m)
            for q in (2, 1, 3, 0):
                gu = quads[q]
                jj, rows = JH * (q % 2) + j, halves[q // 2][1]
                res = _geglu(gu[:, :128], gu[:, 128:], da_v[jj, rows, :].astype(F32))
                for w in range(3):
                    act[w, jj, rows, :] = res[w].astype(BF)
        return carry

    for cp in wgu_copies:
        cp.wait()
    beta_gu(0, 0)
    beta_gu(1, 0)
    gate_step(0, 0, first=True)
    jax.lax.fori_loop(1, NTILE, gate_step, 0)

    def ffn_step(i, carry):
        halves = [half_rows(i, h) for h in range(2)]
        blocks = [[(JH * (q % 2) + j, halves[q // 2][0]) for j in range(JH)] for q in range(4)]
        for k in range(7):
            for part in range(2):
                for t in range(2):
                    lt[0, k, 2 * i + part, 128 * t:128 * t + 128, :] = (
                        ah[i, k, t, Q * part:Q * part + Q, :].astype(F32).T.astype(BF))
        cg, cu = operands(_gamma, 0, blocks, 1), operands(_gamma, 1, blocks, 1)
        summed = [k for k in range(7) if k not in _PLAIN[_alpha]]
        for j in range(JH):
            cs = _alpha(*[act[2, blk[j][0], pl.ds(blk[j][1], H), :].astype(F32) for blk in blocks])
            for n, k in enumerate(summed):
                da_v[j, H * n:H * n + H, :] = cs[k].astype(BF)

        def a_operand(k):
            if k in summed:
                n = summed.index(k)
                return _bf(_cat([da32[j, H // 2 * n:H // 2 * (n + 1), :] for j in range(JH)]))
            return _bf(_cat([act32[2, j, pl.ds(aligned(r // 2, H // 2), H // 2), :] for j, r in blocks[_PLAIN[_alpha][k]]]))

        def ln2_bwd_rows(part, val):
            for r in range(0, Q, R):
                after(dx1_v, (1,), val[2 * r:2 * r + 8])
                rows = pl.ds(pl.multiple_of(2 * H * i + Q * part + r, R), R)
                y1 = y1_v[rows, :]
                dh2 = dx1_v[rows, :]
                rstd = _cat([st2[1, rows, :]] * 4)
                xhat = (x_v[rows, :].astype(F32) + mod_row(2) * y1 - _cat([st2[0, rows, :]] * 4)) * rstd
                dhx = dh2 * xhat
                sums[3] += _colsum8(dh2)
                sums[4] += _colsum8(dhx)
                cb1 = 1.0 + mod_row(4)
                dn = dh2 * cb1
                m1 = _rowsum(_tiles(dn)) * (1.0 / D)
                m2 = _rowsum(_tiles(dhx * cb1)) * (1.0 / D)
                dx1 = do_v[rows, :].astype(F32) + rstd * (dn - m1 - xhat * m2)
                dx1_v[rows, :] = dx1
                sums[2] += _colsum8(dx1 * y1)
            r0 = pl.multiple_of(2 * H * i + Q * part, Q)
            return lambda: d_forward(dx1_v[pl.ds(r0, Q), :] * mod_row(2), r0, (2 * H * i + Q * part) // N2, 1)

        dh, todo = {}, []
        for k in (5, 6, 0, 2, 4, 1, 3):
            pg = _dot_nt(cg[k], _bf(_cat([bgu32[0, k, j] for j in range(JH)])))
            if k in (1, 3):
                todo.append(ln2_bwd_rows(k // 2, pg))
            dh[k] = pg + _dot_nt(cu[k], _bf(_cat([bgu32[1, k, j] for j in range(JH)])))
            if k == 4:
                dx1_v[halves[0][1], :] = _cat([dh[0] + dh[2] + dh[4] - dh[5], dh[4] + dh[6]])
            if k == 3:
                dx1_v[halves[1][1], :] = _cat([dh[1] + dh[5], dh[0] + dh[1] + dh[3] - dh[6]])
        y2 = {}
        for n, k in enumerate((1, 3, 2, 4, 0, 5, 6)):
            y2[k] = _dot(a_operand(k), _bf(_cat([bd32[k, 0], bd32[k, 1]])))
            if n in (0, 1, 3, 5):
                todo.pop(0)()
            if n in (0, 2):
                todo.append(ln2_bwd_rows(2 + n // 2, y2[k]))
        y2 = _gamma_t(y2)
        for q in (2, 1, 3, 0):
            yv = y2[q]
            rows, cols = halves[q // 2][1], slice(256 * (q % 2), 256 * (q % 2) + 256)
            sums[5, :, cols] += _colsum8(do_v[rows, cols].astype(F32) * yv)
            x1 = x_v[rows, cols].astype(F32) + mod_row(2)[:, cols] * y1_v[rows, cols]
            for t, tile in enumerate(_tiles(x1 + mod_row(5)[:, cols] * yv)):
                out_v[2 * (q % 2) + t, rows, :] = tile.astype(BF)
        for cp in row_out(out_v, out_hbm, 0, i):
            cp.start()
        return carry

    jax.lax.fori_loop(0, NTILE, ffn_step, 0)

    radix = spread([f for t, g in groups for f in radix_forward(t, g)], after_obuf, 40)

    def transposed_dy2(i, part):
        dt, db = (do_v[pl.ds(2 * H * i + H * h + Q * part, Q), :].astype(F32) * mod_row(5) for h in range(2))
        for k, v in enumerate(_alpha(dt[:, :256].T, dt[:, 256:].T, db[:, :256].T, db[:, 256:].T)):
            lt[1, k, 2 * i + part] = v.astype(BF)

    lefts = spread([functools.partial(transposed_dy2, i, part) for i in range(NTILE) for part in range(2)],
                   lambda v: after(do_v, (1,), v), 40)
    for n in range(6):
        dwgu_chunk(n, shifted(lambda k, val: (radix(k, val), lefts(k, val)), n))

    def spec_bwd_step(i, carry):
        def pair(pp):
            p = 4 * i + pp
            packed, out = [[], []], []
            for e, (wr, wi) in enumerate(filt(p)):
                a = 2 * p + e
                spec = s_forward(a)
                gr, gi = spec[:N2], spec[N2:]
                xr, xi = xs[a, 0:N2, :], xs[a, N2:2 * N2, :]
                for k, v in enumerate((gr * xr + gi * xi, gi * xr - gr * xi)):
                    packed[k].append(pltpu.bitcast(pltpu.pack_elementwise(_tiles(v), packed_dtype=BF), U32))
                out.append((a, gr * wr + gi * wi, gi * wr - gr * wi))
            for k in range(2):
                for t in range(S // 128):
                    dwq[k, t, pl.ds(pl.multiple_of(8 * p, 8), 8), :] = _cat([v[4 * t:4 * t + 4] for v in packed[k]], 0)
            return out

        pending = pair(0)

        def between(k, val):
            if k in (0, 2, 4):
                pending.extend(pair(k // 2 + 1))
            s_inverse(*pending.pop(0))

        dwgu_chunk(6 + i, between)
        s_inverse(*pending.pop(0))
        return carry

    jax.lax.fori_loop(0, 4, spec_bwd_step, 0, unroll=True)

    def nyq_filter_bwd(gr, gi):
        gr, gi = gr * (1.0 / (S * D)), gi * (1.0 / (S * D))
        for k, grad in enumerate((gr * xn[0] + gi * xn[1], gi * xn[0] - gr * xn[1])):
            own = jnp.where(lane < N1, grad, 0.0)
            flat = own
            for e in range(1, 4):
                flat = jnp.where((sub & 3) == e, pltpu.roll(own, N1 * e, 1), flat)
            pieces = []
            for g in range(N2 // 8):
                blk = flat[8 * g:8 * g + 8]
                pieces += [jnp.sum(jnp.where((sub[:8] < 4) == first, blk, 0.0), axis=0, keepdims=True)
                           for first in (True, False)]
            wri_v[k, 256:257, :] = _cat(pieces).astype(BF)
        return [gr * wn[0] + gi * wn[1], gi * wn[0] - gr * wn[1]]

    side = nyquist(nyq_filter_bwd)
    dwri_copies = [pltpu.make_async_copy(wri_v.at[k], dst, osem.at[10 + k]) for k, dst in enumerate((dwr_hbm, dwi_hbm))]

    def filter_grad(k, t):
        wri_v[k, 0:256, 128 * t:128 * t + 128] = _bf(jnp.take_along_axis(
            dwq[k, t].T, 4 * (lane_d & (N1 - 1)) + (lane_d >> 5), axis=1))

    radix = spread([f for t, g in groups for f in radix_inverse(t, g)], after_vbuf, 26)
    filter_grad(0, 0)
    grads = spread([functools.partial(filter_grad, k, t) for k in range(2) for t in range(S // 128)][1:],
                   lambda v: after(dwq, (0, 0, 0), pltpu.bitcast(v[0:8], U32)), 24)
    for n in range(4):
        dwgu_chunk(10 + n, shifted(lambda k, val: (radix(k, val), grads(k, val), next(side, None)), n))
    for cp in dwri_copies + dwgu_copies:
        cp.start()

    def dh1_rows(i, part):
        r0 = 2 * H * i + Q * part
        y1_v[pl.ds(r0, Q), :] = d_inverse(r0, Q, r0 // N2, 2)

    def ln1_bwd_rows(i, r):
        rows = pl.ds(2 * H * i + r, R)
        dh1 = y1_v[rows, :]
        rstd = _cat([st1[1, rows, :]] * 4)
        xhat = (x_v[rows, :].astype(F32) - _cat([st1[0, rows, :]] * 4)) * rstd
        dhx = dh1 * xhat
        sums[0] += _colsum8(dh1)
        sums[1] += _colsum8(dhx)
        ca1 = 1.0 + mod_row(1)
        dn = dh1 * ca1
        m1 = _rowsum(_tiles(dn)) * (1.0 / D)
        m2 = _rowsum(_tiles(dhx * ca1)) * (1.0 / D)
        for t, tile in enumerate(_tiles(dx1_v[rows, :] + rstd * (dn - m1 - xhat * m2))):
            dx_v[t, rows, :] = tile.astype(BF)

    def ln1_bwd_step(i, carry):
        norms = spread([functools.partial(ln1_bwd_rows, i, r) for r in range(0, 2 * H, R)],
                       lambda v: after(y1_v, (1,), v), 6)

        def between(k, val):
            norms(k, val)
            if k in (0, 1, 3):
                dh1_rows(i, (k + 3) // 2)
            if k == 5 and i + 1 < NTILE:
                dh1_rows(i + 1, 0)

        dwd_chunk(i, between)
        dwd_start(i)
        for cp in row_out(dx_v, dx_hbm, 4, i):
            cp.start()
        return carry

    dh1_rows(0, 0)
    for i in range(NTILE):
        ln1_bwd_step(i, 0)
    dcacc[...] = jnp.zeros(dcacc.shape, F32)

    def dwm_copy(b, t):
        cols = pl.ds(D * b + 128 * t, 128)
        return pltpu.make_async_copy(dwm_v.at[b, t], dwm_hbm.at[:, cols], osem.at[12])

    def mod_grad(b, r):
        dmod = jnp.sum(sums[b], axis=0, keepdims=True).astype(BF).astype(F32)
        sc = scol[r:r + Q, :]
        for t, tile in enumerate(_tiles(dmod)):
            dwm_v[b, t, r:r + Q, :] = (sc * tile).astype(BF)
        prod = _tiles(wm_v[b, r:r + Q, :].astype(F32) * dmod)
        dcacc[r:r + Q, :] += (prod[0] + prod[1]) + (prod[2] + prod[3])

    grads = spread([functools.partial(mod_grad, b, r) for b in range(6) for r in range(0, D, Q)],
                   lambda v: after(sums, (4, 0), v), 12)

    def finish(k, val):
        grads(k, val)
        if k in (2, 4, 6, 8, 10, 12):
            for t in range(4):
                dwm_copy(k // 2 - 1, t).start()
        if k == 13:
            ds = jnp.sum(dcacc[...].T, axis=0, keepdims=True).astype(BF).astype(F32)
            dc_ref[...] = (ds * (sig * (1.0 + cv * (1.0 - sig)))).astype(BF)

    for n in range(JH - NTILE):
        dwd_chunk(NTILE + n, shifted(finish, n))
        dwd_start(NTILE + n)

    for i in range(NTILE):
        for cp in row_out(out_v, out_hbm, 0, i) + row_out(dx_v, dx_hbm, 4, i):
            cp.wait()
    for cp in dwri_copies + dwgu_copies:
        cp.wait()
    for b in range(6):
        for t in range(4):
            dwm_copy(b, t).wait()
    for j in range(JH):
        for half in range(2):
            dwd_copy(j, half).wait()


@jax.jit
def pallas_adaLN_cond__spectral_gfnet__geglu_ffn__prompt_kernel(
    A_x: jax.Array,
    A_w_r: jax.Array,
    A_w_i: jax.Array,
    B_x: jax.Array,
    B_w_gate: jax.Array,
    B_w_up: jax.Array,
    B_w_down: jax.Array,
    c: jax.Array,
    w_mod: jax.Array,
    grad_out: jax.Array,
):
    del B_x
    vm = pltpu.VMEM
    hbm = pl.BlockSpec(memory_space=pl.ANY)
    sds = jax.ShapeDtypeStruct
    scratch = [
        vm((S + 32, D), BF), vm((S + 32, D), BF), vm((2, D // 2 + 1, S), BF), vm((2, D + 64, F), BF),
        vm((F, D), BF), vm((6, D, D), BF), vm((8, 128, 128), BF), vm((N1, 128, 128), BF),
        vm((4, 6, 128, 128), BF), vm((N1, 128, 128), BF), vm((D + 128, 128), F32), vm((8, 8, D), F32),
        vm((2, 7, JH, 256, 128), BF), vm((7, 2, F // 2, 128), BF),
        vm((4, S + 128, 128), F32), vm((2, N1, 128, 128), BF), vm((2, N1 + 1, 128, 128), F32),
        vm((N1, 128, 256), F32), vm((2, S // 128, 128, 128), U32), vm((2, S // 128, 128, 128), U32),
        vm((2, N2, 128), F32), vm((2, N2, 128), F32), vm((N2, 128), F32),
        vm((S + 32, D), F32), vm((2, S, 128), F32), vm((2, S, 128), F32),
        vm((NTILE, 7, 2, H, 128), BF), vm((2, 7, 2 * NTILE, 256, 128), BF), vm((3, 2 * JH, S, 128), BF),
        vm((2 * JH, S, 128), BF), vm((4, S, 128), BF), vm((4, S, 128), BF), vm((S + 32, D), F32), vm((6, 4, D, 128), BF),
        vm((8, 8, D), F32), vm((D, 128), F32),
        pltpu.SMEM(_SPARE.shape, jnp.int32), vm((1, D), BF), vm((2, N2, 128), F32), vm(_MF.shape, F32),
        pltpu.SemaphoreType.DMA((25,)), pltpu.SemaphoreType.DMA((14,)),
    ]
    outs = pl.pallas_call(
        _kernel,
        in_specs=[hbm] * 13,
        out_specs=[hbm] * 7 + [pl.BlockSpec(memory_space=vm), hbm],
        out_shape=[sds((S, D), BF), sds((S, D), BF), sds((D // 2 + 1, S), BF), sds((D // 2 + 1, S), BF), sds((D, F), BF),
                   sds((D, F), BF), sds((F, D), BF), sds((1, D), BF), sds((D, 6 * D), BF)],
        scratch_shapes=scratch,
        compiler_params=pltpu.CompilerParams(vmem_limit_bytes=124 * 2 ** 20),
    )(_SPARE, c, _TWID, A_x.reshape(S, D), grad_out.reshape(S, D), A_w_r.T, A_w_i.T, B_w_gate, B_w_up, B_w_down, w_mod, _DMAT, _MF)
    return (outs[0].reshape(1, S, D), outs[1].reshape(1, S, D), outs[2].T, outs[3].T) + tuple(outs[4:])
```
